```python
import os as _os
_os.environ.setdefault("JAX_PLATFORMS", "cpu")
import jax
import jax.numpy as jnp

def _softmax(x, axis=-1):
    return jax.nn.softmax(x, axis=axis)
def _gelu(x):
    return jax.nn.gelu(x, approximate=True)
def _silu(x):
    return jax.nn.silu(x)
def _sigmoid(x):
    return jax.nn.sigmoid(x)
def _layernorm(x, axis=-1, eps=1e-5):
    m = jnp.mean(x, axis=axis, keepdims=True)
    v = jnp.var(x, axis=axis, keepdims=True)
    return (x - m) / jnp.sqrt(v + eps)
def _scatter_add(tgt, idx, src, axis=0):
    return tgt.at[idx].add(src)
def _segment_sum(src, seg, n):
    return jax.ops.segment_sum(src, seg, n)
class _Rng:
    def __init__(self, key):
        self._k = key
    def _next(self):
        self._k, sub = jax.random.split(self._k)
        return sub
    def normal(self, shape):
        return jax.random.normal(self._next(), shape, dtype=jnp.bfloat16)
    def randint(self, lo, hi, shape):
        return jax.random.randint(self._next(), shape, lo, hi, dtype=jnp.int32)
    def uniform(self, shape, lo=0.0, hi=1.0):
        return jax.random.uniform(self._next(), shape, jnp.bfloat16, lo, hi)
    def permutation(self, n):
        return jax.random.permutation(self._next(), n)


kernel_name = 'interleave_layers__sliding_local_dilated__glu_gated_reglu__prompt'

def setup_inputs():
    _rng = _Rng(jax.random.key(int.from_bytes(__import__("os").urandom(4), "little")))
    _w = (lambda a: (lambda t: t.astype(jnp.bfloat16) if jnp.issubdtype(t.dtype, jnp.floating) else t)(jnp.asarray(a)))
    def _A_setup():
        B, S, D = 1, 2048, 512
        return {
            "x": _w((lambda *s: _rng.normal(s) * 0.05)(B, S, D)),
            "wqkv": _w((lambda *s: _rng.normal(s) * 0.05)(D, 3 * D)),
            "wo": _w((lambda *s: _rng.normal(s) * 0.05)(D, D)),
        }
    _A_in = _A_setup()

    def _B_setup():
        B, S, D, F = 1, 2048, 512, 1792
        return {
            "x": _w((lambda *s: _rng.normal(s) * 0.05)(B, S, D)),
            "W_gate": _w((lambda *s: _rng.normal(s) * 0.8)(D, F) * (2.0 / D) ** 0.5),
            "W_up": _w((lambda *s: _rng.normal(s) * 0.8)(D, F) * (2.0 / D) ** 0.5),
            "W_down": _w((lambda *s: _rng.normal(s) * 0.8)(F, D) * (1.0 / F) ** 0.5),
        }
    _B_in = _B_setup()

    return {
        "A_x": _A_in["x"],
        "A_wqkv": _A_in["wqkv"],
        "A_wo": _A_in["wo"],
        "B_x": _B_in["x"],
        "B_W_gate": _B_in["W_gate"],
        "B_W_up": _B_in["W_up"],
        "B_W_down": _B_in["W_down"],
    }

def reference(A_x, A_wqkv, A_wo, B_x, B_W_gate, B_W_up, B_W_down):
    def _A_ref(x, wqkv, wo):
        B, S, D = x.shape
        H = 32; Dh = D // H
        W, dil = 8, 2
        qkv = (lambda x, *d: x.transpose(*d))((x @ wqkv).reshape(B, S, 3, H, Dh), 2, 0, 3, 1, 4)
        q, k, v = qkv[0], qkv[1], qkv[2]
        scale = Dh ** -0.5
        pos = jnp.arange(S)
        off = jnp.arange(W) * dil
        idx = pos[:, None] - off[None, :]
        mask = idx >= 0
        idx_c = jnp.where(mask, idx, 0).reshape(-1)
        kg = k[:, :, idx_c, :].reshape(B, H, S, W, Dh)
        vg = v[:, :, idx_c, :].reshape(B, H, S, W, Dh)
        logits = jnp.einsum("bhsd,bhswd->bhsw", q, kg) * scale
        logits = jnp.where(mask[None, None, :, :], logits, -1e9)
        attn = _softmax(logits, axis=-1)
        o = jnp.einsum("bhsw,bhswd->bhsd", attn, vg)
        return (lambda x, *d: x.transpose(*d))(o, 0, 2, 1, 3).reshape(B, S, D) @ wo

    def _B_ref(x, W_gate, W_up, W_down):
        gate = jnp.einsum("bsd,df->bsf", x, W_gate)
        up = jnp.einsum("bsd,df->bsf", x, W_up)
        gate = gate * (lambda x, dt: x.astype(dt))(gate > 0, gate.dtype)
        h = gate * up
        return jnp.einsum("bsf,fd->bsd", h, W_down)

    x = A_x
    x = x + _A_ref(_layernorm(x, axis=-1), A_wqkv, A_wo)
    x = x + _B_ref(_layernorm(x, axis=-1), B_W_gate, B_W_up, B_W_down)
    x = x + _A_ref(_layernorm(x, axis=-1), A_wqkv, A_wo)
    x = x + _B_ref(_layernorm(x, axis=-1), B_W_gate, B_W_up, B_W_down)
    return x
```

```python
import functools

import jax
import jax.numpy as jnp
import numpy as np
from jax.experimental import pallas as pl
from jax.experimental.pallas import tpu as pltpu

S, D, F = 2048, 512, 1792
H, DH, W = 32, 16, 8
L = 128
NJ = 8
KB = D // L
R = 16
CH = 64
NCH = 2 * F // 4 // CH
HC = CH // 2
EPS = 1e-5
BF, F32, U32 = jnp.bfloat16, jnp.float32, jnp.uint32
P = functools.partial


def _lo(w):
    return pltpu.bitcast(w << 16, F32)


def _hi(w):
    return pltpu.bitcast(w & np.uint32(0xFFFF0000), F32)


def _halves(w):
    return pltpu.bitcast(w, BF)


def _add(a, b):
    return [[x + y for x, y in zip(ra, rb)] for ra, rb in zip(a, b)]


def _sub(a, b):
    return [[x - y for x, y in zip(ra, rb)] for ra, rb in zip(a, b)]


def _keep(a):
    return a


_LHS = ((_add, 0, 3), (_add, 2, 3), (_keep, 0), (_keep, 3), (_add, 0, 1), (_sub, 2, 0), (_sub, 1, 3))
_RHS = ((_add, 0, 3), (_keep, 0), (_sub, 1, 3), (_sub, 2, 0), (_keep, 3), (_add, 0, 1), (_add, 2, 3))


def _terms(table, grid):
    blocks = [[[b]] for row in grid for b in row]
    return [op(*[blocks[a] for a in args])[0][0] for op, *args in table]


def _products2(product):
    p22 = product(5)
    yield
    m3 = product(2)
    p22 = p22 + m3
    yield
    m5 = product(4)
    c12 = m3 + m5
    yield
    p11 = product(6) - m5
    yield
    m1 = product(0)
    p11, p22 = p11 + m1, p22 + m1
    yield
    m2 = product(1)
    c22 = p22 - m2
    yield
    m4 = product(3)
    yield
    return [[p11 + m4, c12], [m2 + m4, c22]]


def _products4(product, put, get, emit):
    for i in range(7):
        m = yield from _products2(lambda j: product(7 * i + j))
        for r, c in ((0, 1), (1, 1), (1, 0), (0, 0)):
            old = lambda n: get(n, 2 * r + c)
            if i < 5:
                put(i, 2 * r + c, m[r][c])
            if i == 3:
                emit(2 + r, c, m[r][c] + old(1))
            elif i == 4:
                emit(r, 2 + c, m[r][c] + old(2))
            elif i == 5:
                emit(2 + r, 2 + c, m[r][c] + (old(0) - old(1) + old(2)))
            elif i == 6:
                emit(r, c, m[r][c] + (old(0) + old(3) - old(4)))


class _Task:
    def __init__(self, cost, gen):
        self.cost, self.gen = cost, gen

    def take(self, cost):
        cost = min(cost, self.cost)
        self.cost -= cost

        def gen():
            done = 0
            while done < cost:
                step = next(self.gen, None)
                if step is None:
                    return
                done += step
                yield step
        return _Task(cost, gen())


def _chain(*tasks):
    def gen():
        for t in tasks:
            yield from t.gen
    return _Task(sum(t.cost for t in tasks), gen())


def _once(f, *args):
    def gen():
        f(*args)
        yield 0
    return _Task(0, gen())


def _run(main, *sides, lead=0, slack=0):
    side = _chain(*sides)
    now = done = 0
    for step in main.gen:
        now += step
        while done <= side.cost * (now - lead) / (main.cost - lead - slack):
            step = next(side.gen, None)
            if step is None:
                break
            done += step
    for _ in side.gen:
        pass


def _operand_layout():
    layout, row = {}, 0
    for name, (n, rows) in {**{"x%d" % s: (2, 2 * L) for s in range(4)}, "f": (7, L), "o": (2, 2 * L),
                            "h2": (7, 3 * L), "h1": (2, L)}.items():
        layout[name] = (row, rows)
        row += n * rows
    return layout, row + L


def _scratch():
    level1 = pltpu.VMEM((1, 7, 2, 2 * L, L), BF)
    two = lambda s: [s, s]
    return dict(
        xin=pltpu.VMEM((NJ, L, D), U32),
        wqkv_raw=pltpu.VMEM((3, D // 2, D), U32),
        wo_raw=[pltpu.VMEM((1, D // 2, L), U32)] * KB,
        wgu_raw=pltpu.VMEM((2, D // 2, F), U32),
        wd_raw=pltpu.VMEM((F // 2, D), U32),
        zero=pltpu.SMEM((2,), jnp.int32),
        turned=[[pltpu.VMEM((2, KB, L // 2, L), U32)] * 4] * 4,
        wide=[pltpu.VMEM((1, KB + 1, D, L), F32)] * 11,
        wqkv=[level1] * 3, wo=level1,
        wgu=[pltpu.VMEM((1, 49, 1, L, L), BF)] * 7,
        wd2=two([pltpu.VMEM((1, 7, 3, CH, L), BF)] * 7),
        wd1=pltpu.VMEM((1, 7, 1, 2 * L, L), BF),
        xa=pltpu.VMEM((4, 5, D, L), F32),
        xb=pltpu.VMEM((4, 5, D, L), F32),
        stats=pltpu.VMEM((1, 8, 8, L), F32),
        xn=pltpu.VMEM((1, 5, D, L), F32),
        operands=[pltpu.VMEM((1, _operand_layout()[1], L), BF)] * 7,
        q_s=pltpu.VMEM((2, NJ, D, L), F32),
        k_s=pltpu.VMEM((2, 2 * NJ + 1, D, L), F32),
        v_s=pltpu.VMEM((2, 2 * NJ + 1, D, L), F32),
        probs=pltpu.VMEM((1, 16 * W, 8, L), F32),
        o_s=pltpu.VMEM((1, 5, D, L), F32),
        park_m=[pltpu.VMEM((1, 4, CH, L), F32)] * 5,
        park_h=two([pltpu.VMEM((1, 5, HC, L), F32)] * 4),
        xout=pltpu.VMEM((NJ, L, D), U32),
        sems=pltpu.SemaphoreType.DMA((32,)),
    )


def _kernel(x_hbm, wqkv_hbm, wo_hbm, wg_hbm, wu_hbm, wd_hbm, out_hbm, *, cfg,
            xin, wqkv_raw, wo_raw, wgu_raw, wd_raw, zero, turned, wide, wqkv, wo, wgu, wd2, wd1,
            xa, xb, stats, xn, operands, q_s, k_s, v_s, probs, o_s, park_m, park_h, xout, sems):
    layout, _ = _operand_layout()
    full = cfg["mode"] != "loop"
    sem_ids = iter(range(sems.shape[0]))
    copy = lambda src, dst: pltpu.make_async_copy(src, dst, sems.at[next(sem_ids)])
    lanes = lambda i, n=1: pl.ds(i * n * L, n * L)
    strip = lambda k: pl.ds(k * L if isinstance(k, int) else pl.multiple_of(k * L, L), L)
    lane_slice = lambda i: slice(i * L, (i + 1) * L)
    if full:
        cp_x = [copy(x_hbm.bitcast(U32).at[:, j, :], xin.at[j]) for j in range(NJ)]
        cp_qkv = [copy(wqkv_hbm.at[:, lanes(t, KB)], wqkv_raw.bitcast(BF).at[t]) for t in range(3)]
        cp_o = [copy(wo_hbm.at[:, lanes(r)], wo_raw[r].bitcast(BF).at[0]) for r in range(KB)]
        cp_gu = [[copy(w.at[:, cols], wgu_raw.bitcast(BF).at[i, :, cols]) for i, w in enumerate((wg_hbm, wu_hbm))]
                 for cols in (pl.ds(0, 6 * L), pl.ds(6 * L, 8 * L))]
        cp_d = copy(wd_hbm, wd_raw.bitcast(BF))
    cp_out = {(j, k, n): copy(xout.at[j, :, pl.ds(k * L, n * L)], out_hbm.bitcast(U32).at[:, j, pl.ds(k * L, n * L)])
              for j, k, n in [(j, 0, 4) for j in range(4)] + [(j, k, 2) for j in range(4, NJ) for k in (0, 2)]}

    @pl.loop(0, 2)
    def _(i):
        zero[i] = i

    z = zero[0]
    state = dict(buffer=None, slot=0, regions=0)
    results = []

    def pin(*vals):
        if state["buffer"] is not None:
            for v in vals:
                state["slot"] = (state["slot"] + 1) % 8
                rows = pl.ds(operands[0].shape[1] // 2 - 8 * (state["slot"] + 1), 8)
                state["buffer"].bitcast(U32)[0, rows, :] = v if v.dtype == U32 else pltpu.bitcast(v, U32)

    def release(ref):
        ready = [v for t, v in results[-64:] if t <= results[-1][0] - cfg["lag"]]
        if ready:
            spare = (ref.shape[0] - 1, ref.shape[1] - 1, pl.ds(0, 8))
            ref[spare] = ready[-1] if ref.dtype == F32 else pltpu.bitcast(ready[-1], ref.dtype)

    def put(name, i, row, val):
        first, rows = layout[name]
        operands[i % 7][0, pl.ds(first + i // 7 * rows + row, val.shape[0]), :] = val.astype(BF)

    def rhs(name, i):
        first, rows = layout[name]
        state["buffer"] = operands[i % 7]
        return _halves(operands[i % 7].bitcast(U32)[z, pl.ds((first + i // 7 * rows) // 2, rows // 2), :])

    def terms2(table, source, block, store, which=range(7)):
        quadrant = lambda n: [[block(2 * (n // 2) + a, 2 * (n % 2) + b) for b in range(2)] for a in range(2)]
        for i in which:
            op, *args = table[i]
            release(source(args[0]))
            for n, t in enumerate(_terms(table, op(*[quadrant(a) for a in args]))):
                store(7 * i + n, t)
            yield 9 + 8 * len(args)

    TERMS2 = 7 * 9 + 8 * 12

    def store_lhs(dst, i, k, row, t):
        dst[0, i, k, pl.ds(row, R), :] = t.astype(BF)
        if i % 7 == 6:
            pin(dst.bitcast(U32)[z, 0, 0, pl.ds(0, 8), :])

    def head_major(ref, idx, d2):
        w = ref[(*idx[:-1], pl.ds(idx[-1] + d2, 8, stride=8))]
        return jnp.concatenate([_lo(w), _hi(w)], axis=0)

    def turn_square(t):
        def gen():
            for r in (0, 2, 1, 3):
                if t < 3:
                    w = _halves(wqkv_raw[t, :, lanes(r)])
                else:
                    w = jnp.concatenate([head_major(wo_raw[r], (0, k * L // 2), e)
                                         for k in range(KB) for e in range(L // R)]).astype(BF)
                w = pltpu.bitcast(w.T, U32)
                for k in range(KB):
                    turned[t][r][0, k] = w[:, lane_slice(k)]
                yield 30
        return _Task(4 * 30, gen())

    def prep_square(t):
        def rows(r, k, e):
            if t < 3:
                return head_major(turned[t][r], (z, k, 0), e)
            return _halves(turned[t][r][z, k, pl.ds(8 * e, 8), :]).astype(F32)

        def gen():
            for r in range(2):
                for e in range(L // R):
                    for k in range(2):
                        release(turned[t][r])
                        grid = [[rows(2 * a + r, 2 * b + k, e) for b in range(2)] for a in range(2)]
                        for i, term in enumerate(_terms(_LHS, grid)):
                            store_lhs((*wqkv, wo)[t], i, k, r * L + e * R, term)
                        yield 25
        return _Task(4 * L // R * 25, gen())

    def turn_gu(s):
        def gen():
            for k in range(KB):
                for i in range(2):
                    w = _halves(wgu_raw[i, pl.ds(k * L // 2, L // 2), lanes(s, 2)]).T.astype(F32)
                    for e in range(2 * L // 8):
                        wide[s][0, k, pl.ds(R * e + 8 * i, 8), :] = w[8 * e:8 * e + 8]
                    if cfg["tpin"] and k + i:
                        pin(last)
                    last = w[-8:]
                    yield 32
        return _Task(8 * 32, gen())

    def prep_gu(s):
        def gen():
            for c in range(L // CH):
                for e in range(0, CH, R):
                    yield from terms2(_LHS, lambda _: wide[s],
                                      lambda r, k: wide[s][z, k, pl.ds((4 * c + r) * CH + e, R), :],
                                      lambda i, t: store_lhs(wgu[s], i, 0, c * CH + e, t))
        return _Task(L // R * TERMS2, gen())

    def turn_d(t):
        def gen():
            for k in range(4 if t < 3 else 2):
                if t < 3:
                    rows = [pl.ds(((2 + 4 * t + c) * 4 + k) * HC // 2, HC // 2) for c in range(4)]
                else:
                    rows = [pl.ds((4 * c + 2 * k) * HC // 2, HC) for c in range(2)]
                for n in range(2):
                    w = jnp.concatenate([wd_raw[r, lanes(n, 2)] for r in rows], axis=0)
                    wide[7 + t][0, k, lanes(n, 2), :] = _halves(w).T.astype(F32)
                    yield 32
        return _Task((8 if t < 3 else 4) * 32, gen())

    def prep_d2(c):
        def gen():
            for i in range(7):
                for t in range(3):
                    src = wide[7 + t]
                    for e in range(0, CH, R):
                        yield from terms2(_LHS, lambda _: src, lambda r, k: src[z, k, pl.ds((4 * c + r) * CH + e, R), :],
                                          lambda n, term: store_lhs(wd2[c][i], n % 7, t, e, term), (i,))
        return _Task(3 * CH // R * TERMS2, gen())

    def prep_d1():
        def gen():
            for e in range(0, 2 * L, R):
                release(wide[10])
                grid = [[wide[10][z, k, pl.ds(2 * L * r + e, R), :] for k in range(2)] for r in range(2)]
                for i, term in enumerate(_terms(_LHS, grid)):
                    store_lhs(wd1, i, 0, e, term)
                yield 17
        return _Task(2 * L // R * 17, gen())

    def load_x(h):
        def gen():
            for c in range(4):
                for k in range(KB):
                    t = xin[4 * h + c, :, lanes(k)].T
                    xa[h, c, lanes(k), :] = _lo(t)
                    xa[2 + h, c, lanes(k), :] = _hi(t)
                    yield 32
        return _Task(16 * 32, gen())

    def store_out(columns, strips):
        def gen():
            for j in columns:
                for k in strips:
                    release(xa)
                    even, odd = [pltpu.bitcast(xa[z + q + j // 4, j % 4, lanes(k), :].astype(BF).astype(F32), U32)
                                 for q in (0, 2)]
                    words = (even >> 16) | odd
                    pin(words[-8:])
                    xout[j, :, lanes(k)] = words.T
                    yield 80
        return _Task(len(columns) * len(strips) * 80, gen())

    def rhs1(name, src, block):
        def gen():
            for e in range(0, L, R):
                for k in range(2):
                    for c in range(2):
                        release(src)
                        grid = [[block((2 * a + k) * L + e, 2 * b + c) for b in range(2)] for a in range(2)]
                        for i, t in enumerate(_terms(_RHS, grid)):
                            put(name, 7 * c + i, k * L + e, t)
                        yield 25
        return _Task(L // R * 4 * 25, gen())

    def dot(a_ref, i, row, rows, b):
        if isinstance(a_ref, (list, tuple)):
            a_ref, i = a_ref[i // 7], i % 7
        a = jnp.concatenate([_halves(a_ref.bitcast(U32)[z, i, k, pl.ds(row // 2, rows // 2), :])
                             for k in range(a_ref.shape[2])], axis=1)
        res = jnp.dot(a, b, preferred_element_type=F32)
        results.append(((results[-1][0] if results else 0) + a.shape[0] * a.shape[1] // L // 4, res[:8]))
        return res

    def matmul1(a_ref, name, emit):
        cycles = CH * a_ref.shape[2] // 4

        def gen():
            for r0 in range(0, 2 * L, CH):
                for c in range(2):
                    steps = _products2(lambda i: dot(a_ref, i, r0, CH, rhs(name, 7 * c + i)))
                    for _ in range(7):
                        next(steps)
                        yield cycles
                    try:
                        next(steps)
                    except StopIteration as stop:
                        for a, b in ((0, 1), (1, 1), (1, 0), (0, 0)):
                            emit(a * 2 * L + r0, 2 * b + c, stop.value[a][b])
        return _Task(2 * L // CH * 14 * cycles, gen())

    def matmul2(a_ref, row, rows, name, emit):
        def park(n, i, val):
            park_m[n][0, i, pl.ds(0, rows), :] = val

        cycles = rows * layout[name][1] // L // 4
        steps = _products4(lambda i: dot(a_ref, i, row, rows, rhs(name, i)), park,
                           lambda n, i: park_m[n][z, i, pl.ds(0, rows), :], emit)
        return _Task(49 * cycles, (cycles for _ in steps))

    def moments(src, q, done):
        def gen():
            for c in range(4):
                part = lambda k: src[z + q, c, lanes(k), :].reshape(2, L // 16, 8, L)
                for k in range(KB):
                    release(src)
                    t = jnp.sum(part(k), axis=1)
                    acc = t if k == 0 else acc + t
                    pin(acc[1])
                    yield 16
                mean = jnp.sum(acc[0] + acc[1], axis=0, keepdims=True) * (1.0 / D)
                for k in range(KB):
                    release(src)
                    d = part(k) - mean
                    t = jnp.sum(d * d, axis=1)
                    acc = t if k == 0 else acc + t
                    pin(acc[0], acc[1])
                    yield 48
                var = jnp.sum(acc[0] + acc[1], axis=0, keepdims=True) * (1.0 / D)
                for i, t in enumerate((mean, jax.lax.rsqrt(var + EPS))):
                    stats[0, 2 * c + i] = jnp.broadcast_to(t, (8, L))

        def block(r, c, rows=R):
            mean, scale = [stats[z, 2 * c + i][None] for i in range(2)]
            return ((src[z + q, c, pl.ds(r, rows), :].reshape(rows // 8, 8, L) - mean) * scale).reshape(rows, L)

        return _chain(_Task(16 * 64, gen()), done(block))

    def ln_qkv(q, slot):
        return moments(xa, q, lambda block: rhs1("x%d" % slot, xa, block))

    def ln_ffn(q):
        def done(block):
            def gen():
                for c in range(4):
                    for r in range(0, D, L // 2):
                        release(xb)
                        t = block(r, c, L // 2)
                        xn[0, c, pl.ds(r, L // 2), :] = t
                        pin(t[-8:])
                        yield 16
                for e in range(0, L, R):
                    yield from terms2(_RHS, lambda _: xn, lambda k, c: xn[z, c, pl.ds(k * L + e, R), :],
                                      lambda i, t: put("f", i, e, t))
            return _Task(32 * 16 + L // R * TERMS2, gen())
        return moments(xb, q, done)

    def qkv(n, slot, which=(1, 2, 0)):
        refs = q_s, k_s, v_s
        p, j0 = (n >> 1) & 1, 4 * (n & 1)

        def emit(t, r, c, val):
            j = j0 + c
            refs[t][p, j + NJ * (t > 0), pl.ds(r, CH), :] = val
            if t > 0 and (not isinstance(j, int) or j > 0):
                refs[t][p, j, pl.ds(r, CH), :] = pltpu.roll(val, 1, 1)

        return _chain(*[matmul1(wqkv[t], "x%d" % slot, P(emit, t)) for t in which])

    lane = jax.lax.broadcasted_iota(jnp.int32, (8, L), 1)

    def attend(n, u, weights, values):
        p, c, g = (n >> 1) & 1, u % 4, u // 4
        j = 4 * (n & 1) + c
        block = lambda ref, col, d: ref[z + p, col, pl.ds(g * L + 8 * d, R), :].reshape(2, 8, L)
        if weights:
            logit = [None] * W
            for d in range(0, DH, 2):
                release(k_s)
                qv = block(q_s, j, d)
                for w in range(W):
                    t = qv * block(k_s, NJ + j - w, d)
                    logit[w] = (t[0] if d == 0 else logit[w] + t[0]) + t[1]
                pin(logit[d % W], logit[d % W + 1])
                yield 32
            for w in range(c + 1, W):
                logit[w] = jnp.where(lane < (1 if w > c + 4 else 1 - (n & 1)), -1e9 * DH ** 0.5, logit[w])
            m = functools.reduce(jnp.maximum, logit)
            e = [jnp.exp2((t - m) * (DH ** -0.5 * np.log2(np.e))) for t in logit]
            total = (e[0] + e[1] + e[2] + e[3]) + (e[4] + e[5] + e[6] + e[7])
            inv = pl.reciprocal(total, approx=True)
            inv = inv * (2.0 - total * inv)
            e = [t * inv for t in e]
            if not values:
                for w in range(W):
                    probs[0, W * u + w] = e[w]
                inv = probs[z, 0]
            pin(inv)
            yield 48
        if values:
            for d in range(0, DH, 2):
                release(v_s)
                v = [block(v_s, NJ + j - w, d) for w in range(W)]
                if d == 0 and not weights:
                    e = [probs[z, W * u + w] for w in range(W)]
                o = functools.reduce(jnp.add, [e[w][None] * v[w] for w in range(W)])
                o_s[0, c, pl.ds(g * L + 8 * d, R), :] = o.reshape(R, L)
                pin(o[0], o[1])
                yield 32

    def attention(n, units=range(16), weights=True, values=True):
        return _chain(*[_Task(304 * weights + 256 * values, attend(n, u, weights, values)) for u in units])

    def o_terms():
        return rhs1("o", o_s, lambda r, c: o_s[z, c, pl.ds(r, R), :])

    def residual(dst, src, q, r, c, val):
        rows = pl.ds(r, val.shape[0])
        dst[q, c, rows, :] = src[z + q, c, rows, :] + val

    def proj(q):
        return matmul1(wo, "o", P(residual, xb, xa, q))

    def glu(s, r, c, val):
        val = val.reshape(CH // 16, 2, 8, L)
        park_h[s % 2][2 * (r // 2) + c // 2][0, 2 * (r % 2) + c % 2] = (
            jnp.maximum(val[:, 0], 0.0) * val[:, 1]).reshape(HC, L)

    def hidden_terms(s):
        park = park_h[s % 2]

        def gen():
            for e in range(0, HC, R):
                block = lambda r, c: park[2 * (r // 2) + c // 2][z, 2 * (r % 2) + c % 2, pl.ds(e, R), :]
                if s >= 2:
                    for _ in terms2(_RHS, lambda n: park[n], block, lambda i, t: put("h2", i, (s - 2) * HC + e, t)):
                        yield 20
                else:
                    for k in range(2):
                        for c in range(2):
                            release(park[0])
                            grid = [[block(2 * a + k, 2 * b + c) for b in range(2)] for a in range(2)]
                            for i, t in enumerate(_terms(_RHS, grid)):
                                put("h1", 7 * c + i, (2 * s + k) * HC + e, t)
                            yield 35
        return _Task(HC // R * 140, gen())

    def gate_up():
        def gen():
            for s in range(NCH):
                main = matmul2(wgu[s * CH // L], s * CH % L, CH, "f", P(glu, s))
                post = hidden_terms(s - 1) if s else _Task(0, iter(()))
                now = done = 0
                for step in main.gen:
                    now += step
                    while done < post.cost * (now - cfg["post0"]) / (main.cost - cfg["post0"]):
                        done += next(post.gen)
                    yield step
        return _Task(49 * NCH * CH // 4, gen())

    def gu_tail():
        return hidden_terms(NCH - 1)

    def down1(q):
        return matmul1(wd1, "h1", P(residual, xa, xb, q))

    def down2(q, c, r0=0, rows=CH):
        return matmul2(wd2[c], r0, rows, "h2", lambda a, b, val: residual(xa, xa, q, (4 * c + a) * CH + r0, b, val))

    def down(q):
        return _chain(down1(q), down2(q, 0), down2(q, 1))

    def region(*bounds):
        def wrap(f):
            def body(*args):
                results.clear()
                state["buffer"] = None
                f(*args)
            state["regions"] += 1
            with jax.named_scope("region%d" % state["regions"]):
                if len(bounds) == 2:
                    pl.loop(*bounds)(body)
                elif bounds:
                    pl.when(*bounds)(body)
                else:
                    pl.when(z < state["regions"])(body)
        return wrap

    LEAD, SLACK = cfg["lead"], cfg["slack"]

    U1, U2 = cfg["u1"], cfg["u2"]

    def second_half(m):
        _run(_chain(down1((m - 1) & 3), down2((m - 1) & 3, 0)),
             gu_tail(), attention(m, range(U1 + U2, 16)), o_terms(), lead=LEAD, slack=SLACK)
        _run(proj(m & 3), attention(m + 1, range(U1)))
        _run(down2((m - 1) & 3, 1), ln_ffn(m & 3), lead=LEAD)

    def first_half(m):
        _run(gate_up(), ln_qkv((m - 1) & 3, 0), attention(m + 1, range(U1, U1 + U2)), lead=LEAD)

    def step(m):
        region(m > 0)(P(second_half, m))
        region()(P(first_half, m))
        region((m > 0) & (m < 5))(lambda: _run(qkv(m + 3, 0)))

    def wait(*copies):
        with jax.named_scope("region_wait"):
            for c in copies:
                c.wait()
        results.clear()
        state["buffer"] = None


    def first():
        for c in [*cp_x[:4], *cp_qkv, *cp_x[4:], *cp_o, *cp_gu[0], *cp_gu[1], cp_d]:
            c.start()
        wait(*cp_x[:4])
        _run(load_x(0))
        norm = ln_qkv(0, 0)
        _run(norm.take(cfg["n0"]))
        wait(cp_qkv[0])
        _run(_chain(turn_square(0), norm, prep_square(0)))
        _run(qkv(0, 0, (0,)), ln_qkv(2, 2), lead=LEAD, slack=SLACK)
        wait(*cp_qkv[1:])
        _run(_chain(turn_square(1), turn_square(2)))
        _run(qkv(2, 2, (0,)), prep_square(1), lead=2 * LEAD, slack=SLACK)
        _run(qkv(0, 0, (1,)), prep_square(2))
        wait(*cp_x[4:], *cp_o)
        _run(_chain(load_x(1), turn_square(3)))
        _run(qkv(0, 0, (2,)), ln_qkv(1, 1), lead=cfg["l1"], slack=SLACK)
        _run(qkv(1, 1, (1,)), ln_qkv(3, 3), prep_square(3))

    def second():
        wait(*cp_gu[0])
        preps = _chain(*[prep_gu(s) for s in range(3)])
        b0, b1, b2, b3 = cfg["b"]
        _run(qkv(1, 1, (0,)), turn_gu(0), turn_gu(1), turn_gu(2), preps.take(b0))
        _run(qkv(1, 1, (2,)), preps.take(b1))
        qk = attention(0, values=False)
        pv = attention(0, weights=False)
        mix = lambda att, n, amount: [t for i in range(n) for t in (preps.take(amount // n), att.take(att.cost // (n - i)))]
        _run(_chain(qkv(2, 2, (2,)), qkv(3, 3, (2,))), *mix(qk, 4, b2))
        _run(_chain(qkv(2, 2, (1,)), qkv(3, 3, (1,))), *mix(pv, 4, preps.cost), preps, o_terms(), lead=LEAD)

    def third():
        wait(*cp_gu[1], cp_d)
        _run(proj(0), *[turn_gu(s) for s in range(3, 7)])
        _run(qkv(3, 3, (0,)), turn_d(3), ln_ffn(0), *[turn_d(t) for t in range(cfg["td"])])
        _run(_chain(*[turn_d(t) for t in range(cfg["td"], 3)]))

    def fourth():
        att = attention(1, range(U1))
        preps = _chain(*[prep_gu(s) for s in range(3, 7)], prep_d1(), prep_d2(0), prep_d2(1))
        _run(_chain(*[t for i in range(U1) for t in (preps.take(preps.cost // (U1 - i)), att.take(att.cost // (U1 - i)))],
                    preps, att))

    def last0():
        _run(_chain(down1(3), down2(3, 0)), gu_tail(), store_out(range(4), range(KB)), lead=LEAD, slack=400)
        for j in range(4):
            cp_out[j, 0, 4].start()

    def last1():
        _run(down2(3, 1), store_out(range(4, NJ), (0, 1)), slack=1000)
        results.clear()
        state["buffer"] = None
        _run(store_out((4,), (2, 3)))
        for key in [(j, 0, 2) for j in range(4, NJ)] + [(4, 2, 2)]:
            cp_out[key].start()

    def last2():
        _run(store_out((5, 6, 7), (2, 3)))
        for j in (5, 6, 7):
            cp_out[j, 2, 2].start()

    if cfg["mode"] == "full":
        region()(first)
        region()(second)
        region()(third)
        region()(fourth)
        with jax.named_scope("region_loop"):
            pl.loop(0, 8)(step)
        for f in (last0, last1, last2):
            region()(f)
    else:
        if cfg["mode"] == "loop":
            pl.loop(0, cfg["n"])(step)
        else:
            for f in dict(first=[first], second=[second, third, fourth], last=[last0, last1, last2])[cfg["mode"]]:
                region()(f)
        keep = [q_s, k_s, v_s, xa, xb, o_s, *wide]
        keep = [pltpu.bitcast(r[z, 0, pl.ds(0, 8), :], U32) for r in keep] + [
            r.bitcast(U32)[z, 0, 0, pl.ds(0, 8), :] for r in [*wqkv, wo, *wgu, *wd2[0], *wd2[1], wd1]]
        xout[0, 0:8, 0:L] = functools.reduce(jnp.add, keep)
        if cfg["mode"] == "first":
            wait(*cp_gu[0], *cp_gu[1], cp_d)
        if cfg["mode"] != "last":
            for c in cp_out.values():
                c.start()
    for c in cp_out.values():
        c.wait()


def make(flags=None, **kw):
    cfg = dict(mode="full", post0=256, lag=190, n=8, split=3500, lead=200, slack=100, tpin=False, u1=3, u2=8, b=(600, 1900, 700, 600), td=0, l1=900, n0=1024, ld2=True)
    cfg.update(kw)

    @jax.jit
    def fn(A_x, A_wqkv, A_wo, B_x, B_W_gate, B_W_up, B_W_down):
        del B_x
        any_spec = pl.BlockSpec(memory_space=pl.ANY)
        out = pl.pallas_call(
            functools.partial(_kernel, cfg=cfg),
            out_shape=jax.ShapeDtypeStruct((L, 2 * NJ, D), BF),
            in_specs=[any_spec] * 6,
            out_specs=any_spec,
            scratch_shapes=_scratch(),
            compiler_params=pltpu.CompilerParams(vmem_limit_bytes=120 * 2**20, flags=flags,
                                                 disable_semaphore_checks=True, disable_bounds_checks=cfg.get("nobc", True)),
            name="fused_layers",
        )(A_x.reshape(L, 2 * NJ, D), A_wqkv, A_wo, B_W_gate, B_W_up, B_W_down)
        return out.reshape(1, S, D)
    return fn


pallas_interleave_layers__sliding_local_dilated__glu_gated_reglu__prompt_kernel = make()
```

```python
import functools

import jax
import jax.numpy as jnp
import numpy as np
from jax.experimental import pallas as pl
from jax.experimental.pallas import tpu as pltpu

S, D, F = 2048, 512, 1792
DH, W = 16, 8
L = 128
NJ = 8
KB = D // L
R = 16
CH = 64
NCH = 2 * F // 4 // CH
HC = CH // 2
EPS = 1e-5
LAG = 180
TERMS2 = 7 * 9 + 8 * 12
EARLY = 11
BF, F32, U32 = jnp.bfloat16, jnp.float32, jnp.uint32
P = functools.partial


def _lo(words):
    return pltpu.bitcast(words << 16, F32)


def _hi(words):
    return pltpu.bitcast(words & np.uint32(0xFFFF0000), F32)


def _halves(words):
    return pltpu.bitcast(words, BF)


def _lanes(i, n=1):
    return pl.ds(i * n * L, n * L)


def _aligned(row):
    return row if isinstance(row, int) else pl.multiple_of(row, R)


def _add(a, b):
    return [[x + y for x, y in zip(ra, rb)] for ra, rb in zip(a, b)]


def _sub(a, b):
    return [[x - y for x, y in zip(ra, rb)] for ra, rb in zip(a, b)]


def _keep(a):
    return a


_LHS = ((_add, 0, 3), (_add, 2, 3), (_keep, 0), (_keep, 3), (_add, 0, 1), (_sub, 2, 0), (_sub, 1, 3))
_RHS = ((_add, 0, 3), (_keep, 0), (_sub, 1, 3), (_sub, 2, 0), (_keep, 3), (_add, 0, 1), (_add, 2, 3))


def _terms(table, grid):
    blocks = [[[b]] for row in grid for b in row]
    return [op(*[blocks[a] for a in args])[0][0] for op, *args in table]


def _products2(product):
    p22 = product(5)
    yield
    m3 = product(2)
    p22 = p22 + m3
    yield
    m5 = product(4)
    c12 = m3 + m5
    yield
    p11 = product(6) - m5
    yield
    m1 = product(0)
    p11, p22 = p11 + m1, p22 + m1
    yield
    m2 = product(1)
    c22 = p22 - m2
    yield
    m4 = product(3)
    yield
    return [[p11 + m4, c12], [m2 + m4, c22]]


def _products4(product, put, get, emit):
    for i in range(7):
        m = yield from _products2(lambda j: product(7 * i + j))
        for r, c in ((0, 1), (1, 1), (1, 0), (0, 0)):
            old = lambda n: get(n, 2 * r + c)
            if i < 5:
                put(i, 2 * r + c, m[r][c])
            if i == 3:
                emit(2 + r, c, m[r][c] + old(1))
            elif i == 4:
                emit(r, 2 + c, m[r][c] + old(2))
            elif i == 5:
                emit(2 + r, 2 + c, m[r][c] + (old(0) - old(1) + old(2)))
            elif i == 6:
                emit(r, c, m[r][c] + (old(0) + old(3) - old(4)))


class _Task:
    def __init__(self, cost, gen):
        self.cost, self.gen = cost, gen

    def take(self, cost):
        cost = min(cost, self.cost)
        self.cost -= cost
        if self.cost == 0:
            return _Task(cost, self.gen)

        def gen():
            done = 0
            while done < cost:
                step = next(self.gen, None)
                if step is None:
                    return
                done += step
                yield step
        return _Task(cost, gen())


def _chain(*tasks):
    def gen():
        for t in tasks:
            yield from t.gen
    return _Task(sum(t.cost for t in tasks), gen())


def _run(main, *sides, lead=0, slack=0):
    side = _chain(*sides)
    now = done = 0
    for step in main.gen:
        now += step
        while done <= side.cost * (now - lead) / (main.cost - lead - slack):
            step = next(side.gen, None)
            if step is None:
                break
            done += step
    for _ in side.gen:
        pass


def _operand_layout():
    layout, row = {}, 0
    for name, (n, rows) in {**{"x%d" % s: (2, 2 * L) for s in range(4)}, "f": (7, L), "o": (2, 2 * L),
                            "h2": (7, 3 * L), "h1": (2, L)}.items():
        layout[name] = (row, rows)
        row += n * rows
    return layout, row + L


def _scratch():
    level1 = pltpu.VMEM((1, 7, 2, 2 * L, L), BF)
    return dict(
        xin=pltpu.VMEM((NJ, L, D), U32),
        wqkv_raw=pltpu.VMEM((3, D // 2, D), U32),
        wo_raw=[pltpu.VMEM((1, D // 2, L), U32)] * KB,
        wgu_raw=pltpu.VMEM((2, D // 2, F), U32),
        wd_raw=pltpu.VMEM((F // 2, D), U32),
        zero=pltpu.SMEM((2,), jnp.int32),
        turned=[[pltpu.VMEM((2, KB, L // 2, L), U32)] * 4] * 4,
        turned_ffn=[pltpu.VMEM((n, KB + 1, D // 2, L), U32) for n in (1, 1, 1, 4, 3, 1)],
        wqkv=[level1] * 3,
        wo=level1,
        wgu=pltpu.VMEM((7, 49, 1, L, L), BF),
        wd2=pltpu.VMEM((2, 49, 3, CH, L), BF),
        wd1=pltpu.VMEM((1, 7, 1, 2 * L, L), BF),
        xa=pltpu.VMEM((4, 5, D, L), F32),
        xb=pltpu.VMEM((4, 5, D, L), F32),
        stats=[pltpu.VMEM((1, 2, 8, L), F32)] * 4,
        xn=pltpu.VMEM((1, 5, D, L), F32),
        operands=[pltpu.VMEM((1, _operand_layout()[1], L), BF)] * 7,
        q_s=pltpu.VMEM((2, NJ, D, L), F32),
        k_s=pltpu.VMEM((2, 2 * NJ + 1, D, L), F32),
        v_s=pltpu.VMEM((2, 2 * NJ + 1, D, L), F32),
        probs=pltpu.VMEM((1, 16 * W, 8, L), F32),
        o_s=pltpu.VMEM((1, 5, D, L), F32),
        park_m=[pltpu.VMEM((1, 4, CH, L), F32)] * 5,
        park_h=[[pltpu.VMEM((1, 5, HC, L), F32)] * 4] * 2,
        xout=pltpu.VMEM((NJ, L, D), U32),
        sems=pltpu.SemaphoreType.DMA((36,)),
    )


def _kernel(x_hbm, wqkv_hbm, wo_hbm, wg_hbm, wu_hbm, wd_hbm, out_hbm, *,
            xin, wqkv_raw, wo_raw, wgu_raw, wd_raw, zero, turned, turned_ffn, wqkv, wo, wgu, wd2, wd1,
            xa, xb, stats, xn, operands, q_s, k_s, v_s, probs, o_s, park_m, park_h, xout, sems):
    layout, _ = _operand_layout()
    sem_ids = iter(range(sems.shape[0]))
    copy = lambda src, dst: pltpu.make_async_copy(src, dst, sems.at[next(sem_ids)])
    cp_x = [copy(x_hbm.bitcast(U32).at[:, j, :], xin.at[j]) for j in range(NJ)]
    cp_qkv = [copy(wqkv_hbm.at[:, _lanes(t, KB)], wqkv_raw.bitcast(BF).at[t]) for t in range(3)]
    cp_o = [copy(wo_hbm.at[:, _lanes(r)], wo_raw[r].bitcast(BF).at[0]) for r in range(KB)]
    cp_gu = [[copy(w.at[:, cols], wgu_raw.bitcast(BF).at[i, :, cols]) for i, w in enumerate((wg_hbm, wu_hbm))]
             for cols in (pl.ds(0, 6 * L), pl.ds(6 * L, 8 * L))]
    cp_d = copy(wd_hbm, wd_raw.bitcast(BF))
    pieces = [(j, 0, 4) for j in range(4)] + [(j, k, n) for j in range(4, NJ) for k, n in ((0, 2), (2, 1), (3, 1))]
    cp_out = {(j, k): copy(xout.at[j, :, pl.ds(k * L, n * L)], out_hbm.bitcast(U32).at[:, j, pl.ds(k * L, n * L)])
              for j, k, n in pieces}

    @pl.loop(0, 2)
    def _(i):
        zero[i] = i

    z = zero[0]
    state = dict(buffer=None, slot=0, regions=0)
    results = []

    def pin(*vals):
        if state["buffer"] is not None:
            for v in vals:
                state["slot"] = (state["slot"] + 1) % 8
                rows = pl.ds(operands[0].shape[1] // 2 - 8 * (state["slot"] + 1), 8)
                state["buffer"].bitcast(U32)[0, rows, :] = v if v.dtype == U32 else pltpu.bitcast(v, U32)

    def release(ref):
        ready = [v for t, v in results[-64:] if t <= results[-1][0] - LAG]
        if ready:
            spare = (ref.shape[0] - 1, ref.shape[1] - 1, pl.ds(0, 8))
            ref[spare] = ready[-1] if ref.dtype == F32 else pltpu.bitcast(ready[-1], ref.dtype)

    def untie():
        results.clear()
        state["buffer"] = None

    def put(name, i, row, val):
        first, rows = layout[name]
        operands[i % 7][0, pl.ds(_aligned(first + i // 7 * rows + row), val.shape[0]), :] = val.astype(BF)

    def rhs(name, i):
        first, rows = layout[name]
        state["buffer"] = operands[i % 7]
        return _halves(operands[i % 7].bitcast(U32)[z, pl.ds((first + i // 7 * rows) // 2, rows // 2), :])

    def terms2(table, source, block, store):
        quadrant = lambda n: [[block(2 * (n // 2) + a, 2 * (n % 2) + b) for b in range(2)] for a in range(2)]
        for i, (op, *args) in enumerate(table):
            release(source(args[0]))
            for n, t in enumerate(_terms(table, op(*[quadrant(a) for a in args]))):
                store(7 * i + n, t)
            yield 9 + 8 * len(args)

    def store_lhs(dst, i, k, row, t, slot=0):
        dst[slot, i, k, pl.ds(row, R), :] = t.astype(BF)
        if i % 7 == 6:
            pin(dst.bitcast(U32)[z, 0, 0, pl.ds(0, 8), :])

    def head_major(ref, lead, first, d2):
        w = ref[(*lead, pl.ds(first + d2, 8, stride=8))]
        return jnp.concatenate([_lo(w), _hi(w)], axis=0)

    def turn_square(t):
        def gen():
            for r in (0, 2, 1, 3):
                if t < 3:
                    w = _halves(wqkv_raw[t, :, _lanes(r)])
                else:
                    w = jnp.concatenate([head_major(wo_raw[r], (0,), k * L // 2, e)
                                         for k in range(KB) for e in range(L // R)]).astype(BF)
                w = pltpu.bitcast(w.T, U32)
                for k in range(KB):
                    turned[t][r][0, k] = w[:, k * L:(k + 1) * L]
                yield 30
        return _Task(4 * 30, gen())

    def prep_square(t):
        def rows(r, k, e):
            if t < 3:
                return head_major(turned[t][r], (z, k), 0, e)
            return _halves(turned[t][r][z, k, pl.ds(8 * e, 8), :]).astype(F32)

        def gen():
            for r in range(2):
                for e in range(L // R):
                    for k in range(2):
                        release(turned[t][r])
                        grid = [[rows(2 * a + r, 2 * b + k, e) for b in range(2)] for a in range(2)]
                        for i, term in enumerate(_terms(_LHS, grid)):
                            store_lhs((*wqkv, wo)[t], i, k, r * L + e * R, term)
                        yield 25
        return _Task(4 * L // R * 25, gen())

    def turned_gu(s):
        return (turned_ffn[s], 0) if s < 3 else (turned_ffn[3], s - 3)

    def turn_gu(s):
        def gen():
            dst, slot = turned_gu(s)
            for k in range(KB):
                for i in range(2):
                    w = _halves(wgu_raw[i, pl.ds(k * L // 2, L // 2), _lanes(s, 2)])
                    dst[slot, k, _lanes(i), :] = pltpu.bitcast(w.T, U32)
                    yield 32
        return _Task(8 * 32, gen())

    def prep_level2(src, block, store):
        def gen():
            for c in range(L // CH):
                for e in range(0, CH, R):
                    get = P(block, c, e) if results else functools.cache(P(block, c, e))
                    yield from terms2(_LHS, lambda _: src, get, P(store, c, e))
        return _Task(L // R * TERMS2, gen())

    def prep_gu(s):
        src, slot = turned_gu(s)

        def block(c, e, r, k):
            word, half = (4 * c + r) * HC // 2 + e // 32 * 8, e % 32 // 2
            return jnp.concatenate([
                _halves(src[z + slot, k, pl.ds(i * L + word, 8), :]).astype(F32)[half:half + 8] for i in range(2)])
        return prep_level2(src, block, lambda c, e, i, t: store_lhs(wgu, i, 0, c * CH + e, t, s))

    def turn_d(t):
        def gen():
            dst, slot = (turned_ffn[4], t) if t < 3 else (turned_ffn[5], 0)
            for k in range(4 if t < 3 else 2):
                if t < 3:
                    rows = [pl.ds(((1 + 4 * t + c) * 4 + k) * HC // 2, HC // 2) for c in range(4)]
                else:
                    rows = [pl.ds((4 * c + 2 * k) * HC // 2, HC) for c in (0, NCH - 1)]
                for n in range(2):
                    w = jnp.concatenate([wd_raw[r, _lanes(n, 2)] for r in rows], axis=0)
                    dst[slot, k, _lanes(n), :] = pltpu.bitcast(_halves(w).T, U32)
                    yield 32
        return _Task((8 if t < 3 else 4) * 32, gen())

    def prep_d2(t):
        def block(c, e, r, k):
            row = (2 * c + e // HC) * L + r * HC + e % HC
            return _halves(turned_ffn[4][z + t, k, pl.ds(row // 2, 8), :]).astype(F32)
        return prep_level2(turned_ffn[4], block, lambda c, e, i, term: store_lhs(wd2, i, t, e, term, c))

    def prep_d1():
        def gen():
            for e in range(0, 2 * L, R):
                release(turned_ffn[5])
                grid = [[_halves(turned_ffn[5][z, k, pl.ds(L * r + e // 2, 8), :]).astype(F32)
                         for k in range(2)] for r in range(2)]
                for i, term in enumerate(_terms(_LHS, grid)):
                    store_lhs(wd1, i, 0, e, term)
                yield 17
        return _Task(2 * L // R * 17, gen())

    def load_x(half, columns=(0, 2, 1, 3)):
        for c in columns:
            for k in range(KB):
                t = xin[4 * half + c, :, _lanes(k)].T
                xa[half, c, _lanes(k), :] = _lo(t)
                xa[2 + half, c, _lanes(k), :] = _hi(t)

    def store_out(columns, strips):
        def gen():
            for j in columns:
                for k in strips:
                    release(xa)
                    even, odd = [pltpu.bitcast(xa[z + q + j // 4, j % 4, _lanes(k), :].astype(BF).astype(F32), U32)
                                 for q in (0, 2)]
                    words = (even >> 16) | odd
                    pin(words[-8:])
                    xout[j, :, _lanes(k)] = words.T
                    yield 80
        return _Task(len(columns) * len(strips) * 80, gen())

    def rhs1(name, src, block, c):
        def gen():
            for e in range(0, 2 * L, R):
                release(src)
                grid = [[block(2 * a * L + e, 2 * b + c) for b in range(2)] for a in range(2)]
                for i, t in enumerate(_terms(_RHS, grid)):
                    put(name, 7 * c + i, e, t)
                yield 25
        return _Task(2 * L // R * 25, gen())

    def dot(a_ref, slot, i, row, rows, b):
        a = jnp.concatenate([_halves(a_ref.bitcast(U32)[slot, i, k, pl.ds(row // 2, rows // 2), :])
                             for k in range(a_ref.shape[2])], axis=1)
        res = jnp.dot(a, b, preferred_element_type=F32)
        results.append(((results[-1][0] if results else 0) + a.shape[0] * a.shape[1] // L // 4, res[:8]))
        return res

    def matmul1(a_ref, name, emit, pairs=(0, 1)):
        cycles = CH * a_ref.shape[2] // 4

        def gen():
            for r0 in range(0, 2 * L, CH):
                for c in pairs:
                    steps = _products2(lambda i: dot(a_ref, z, i, r0, CH, rhs(name, 7 * c + i)))
                    for _ in range(7):
                        next(steps)
                        yield cycles
                    try:
                        next(steps)
                    except StopIteration as stop:
                        for a, b in ((0, 1), (1, 1), (1, 0), (0, 0)):
                            emit(a * 2 * L + r0, 2 * b + c, stop.value[a][b])
        return _Task(2 * L // CH * 7 * len(pairs) * cycles, gen())

    def matmul2(a_ref, slot, row, rows, name, emit):
        def park(n, i, val):
            park_m[n][0, i, pl.ds(0, rows), :] = val

        cycles = rows * layout[name][1] // L // 4
        steps = _products4(lambda i: dot(a_ref, slot, i, row, rows, rhs(name, i)), park,
                           lambda n, i: park_m[n][z, i, pl.ds(0, rows), :], emit)
        return _Task(49 * cycles, (cycles for _ in steps))

    def moments(src, q, c):
        def gen():
            part = lambda k: src[z + q, c, _lanes(k), :].reshape(2, L // 16, 8, L)
            for k in range(KB):
                release(src)
                t = jnp.sum(part(k), axis=1)
                acc = t if k == 0 else acc + t
                pin(acc[1])
                yield 16
            mean = jnp.sum(acc[0] + acc[1], axis=0, keepdims=True) * (1.0 / D)
            for k in range(KB):
                release(src)
                d = part(k) - mean
                t = jnp.sum(d * d, axis=1)
                acc = t if k == 0 else acc + t
                pin(acc[0], acc[1])
                yield 48
            var = jnp.sum(acc[0] + acc[1], axis=0, keepdims=True) * (1.0 / D)
            for i, t in enumerate((mean, jax.lax.rsqrt(var + EPS))):
                stats[c][0, i] = jnp.broadcast_to(t, (8, L))
        return _Task(KB * 64, gen())

    def normalized(src, q, r, c, rows=R):
        x = src[z + q, c, pl.ds(r, rows), :].reshape(rows // 8, 8, L)
        return ((x - stats[c][z, 0][None]) * stats[c][z, 1][None]).reshape(rows, L)

    def ln_qkv(q, slot):
        m = [moments(xa, q, c) for c in range(4)]
        t = [rhs1("x%d" % slot, xa, P(normalized, xa, q), c) for c in range(2)]
        return _chain(m[0], m[2], m[1], t[0].take(200), m[3], t[0], t[1])

    def ln_pair(q, c):
        return _chain(moments(xa, q, c), moments(xa, q, c + 2), rhs1("x%d" % q, xa, P(normalized, xa, q), c))

    def ln_ffn(q):
        def scale(c):
            for r in range(0, D, L // 2):
                release(xb)
                t = normalized(xb, q, r, c, L // 2)
                xn[0, c, pl.ds(r, L // 2), :] = t
                pin(t[-8:])
                yield 16

        def terms():
            for e in range(0, L, R):
                yield from terms2(_RHS, lambda _: xn, lambda k, c: xn[z, c, pl.ds(k * L + e, R), :],
                                  lambda i, t: put("f", i, e, t))

        m = [moments(xb, q, c) for c in range(4)]
        n = [_Task(8 * 16, scale(c)) for c in range(4)]
        return _chain(m[0], m[1], m[2], n[0], m[3], n[1], n[2], n[3], _Task(L // R * TERMS2, terms()))

    Q, K, V = range(3)

    def qkv(n, slot, which, shifted=True, pairs=(0, 1)):
        refs = q_s, k_s, v_s
        p, j0 = (n >> 1) & 1, 4 * (n & 1)

        def emit(t, r, c, val):
            j = j0 + c
            refs[t][p, j + NJ * (t > 0), pl.ds(r, CH), :] = val
            if shifted and t > 0 and (not isinstance(j, int) or j > 0):
                refs[t][p, j, pl.ds(r, CH), :] = pltpu.roll(val, 1, 1)

        return _chain(*[matmul1(wqkv[t], "x%d" % slot, P(emit, t), pairs) for t in which])

    def shift(ref, columns):
        def gen():
            for j in columns:
                for r in range(0, D, CH):
                    ref[0, j, pl.ds(r, CH), :] = pltpu.roll(ref[0, NJ + j, pl.ds(r, CH), :], 1, 1)
                    yield 8
        return _Task(len(columns) * D // CH * 8, gen())

    lane = jax.lax.broadcasted_iota(jnp.int32, (8, L), 1)

    def attend(n, u, weights, values, g0):
        p, c, g = (n >> 1) & 1, (0, 2, 1, 3)[u // 4], u % 4 + g0
        j = 4 * (n & 1) + c
        block = lambda ref, col, d: ref[z + p, col, pl.ds(_aligned(g * L + 8 * d), R), :].reshape(2, 8, L)
        if weights:
            logit = [None] * W
            for d in range(0, DH, 2):
                release(k_s)
                qv = block(q_s, j, d)
                for w in range(W):
                    t = qv * block(k_s, NJ + j - w, d)
                    logit[w] = (t[0] if d == 0 else logit[w] + t[0]) + t[1]
                pin(*[logit[(2 * d + i) % W] for i in range(4)])
                yield 32
            for w in range(c + 1, W):
                logit[w] = jnp.where(lane < (1 if w > c + 4 else 1 - (n & 1)), -1e9 * DH ** 0.5, logit[w])
            m = functools.reduce(jnp.maximum, logit)
            e = [jnp.exp2((t - m) * (DH ** -0.5 * np.log2(np.e))) for t in logit]
            total = (e[0] + e[1] + e[2] + e[3]) + (e[4] + e[5] + e[6] + e[7])
            inv = pl.reciprocal(total, approx=True)
            inv = inv * (2.0 - total * inv)
            e = [t * inv for t in e]
            if not values:
                for w in range(W):
                    probs[0, W * u + w] = e[w]
                inv = probs[z, 0]
            pin(inv)
            yield 48
        if values:
            for d in range(0, DH, 2):
                release(v_s)
                v = [block(v_s, NJ + j - w, d) for w in range(W)]
                if d == 0 and not weights:
                    e = [probs[z, W * u + w] for w in range(W)]
                o = functools.reduce(jnp.add, [e[w][None] * v[w] for w in range(W)])
                o_s[0, c, pl.ds(_aligned(g * L + 8 * d), R), :] = o.reshape(R, L)
                pin(o_s[z, 0, pl.ds(0, 8), :])
                yield 32

    def attention(n, units=range(16), weights=True, values=True, g0=0):
        return _chain(*[_Task(304 * weights + 256 * values, attend(n, u, weights, values, g0)) for u in units])

    def o_terms():
        return _chain(*[rhs1("o", o_s, lambda r, c: o_s[z, c, pl.ds(r, R), :], c) for c in range(2)])

    def residual(dst, src, q, r, c, val):
        rows = pl.ds(r, val.shape[0])
        dst[q, c, rows, :] = src[z + q, c, rows, :] + val

    def proj(q):
        return matmul1(wo, "o", P(residual, xb, xa, q))

    def glu(s, r, c, val):
        val = val.reshape(CH // 16, 2, 8, L)
        park_h[s % 2][2 * (r // 2) + c // 2][0, 2 * (r % 2) + c % 2] = (
            jnp.maximum(val[:, 0], 0.0) * val[:, 1]).reshape(HC, L)

    def hidden_terms(s, base=0):
        park = park_h[s % 2]

        def gen():
            for e in range(0, HC, R):
                block = lambda r, c: park[2 * (r // 2) + c // 2][z, 2 * (r % 2) + c % 2, pl.ds(e, R), :]
                if 0 < s < NCH - 1:
                    for _ in terms2(_RHS, lambda n: park[n], block,
                                    lambda i, t: put("h2", i, (base + s - 1) * HC + e, t)):
                        yield 20
                else:
                    for k in range(2):
                        for c in range(2):
                            release(park[0])
                            grid = [[block(2 * a + k, 2 * b + c) for b in range(2)] for a in range(2)]
                            for i, t in enumerate(_terms(_RHS, grid)):
                                put("h1", 7 * c + i, (2 * (s > 0) + k) * HC + e, t)
                            yield 35
        return _Task(HC // R * 140, gen())

    def gate_up(chunks=range(NCH), base=0):
        def gen():
            for s in chunks:
                main = matmul2(wgu, z + (base >> 1) + s * CH // L, s * CH % L, CH, "f", P(glu, s))
                post = hidden_terms(s - 1, base) if s > 0 else _Task(0, iter(()))
                now = done = 0
                for step in main.gen:
                    now += step
                    while done < post.cost * (now - 224) / (main.cost - 224):
                        done += next(post.gen)
                    yield step
        return _Task(49 * len(chunks) * CH // 4, gen())

    def down2(q, first, n=2):
        def emit(a, b, val):
            for i in range(n):
                residual(xa, xa if first else xb, q, (first + i) * L + a * HC, b, val[i * HC:(i + 1) * HC])
        return matmul2(wd2, z + first // 2, first % 2 * HC, n * HC, "h2", emit)

    def down1(q):
        return matmul1(wd1, "h1", lambda r, c, val: residual(xa, xa if r < 2 * L else xb, q, r, c, val))

    def region(when=None, times=None):
        def wrap(f):
            def body(*args):
                untie()
                f(*args)
            state["regions"] += 1
            if times:
                pl.loop(0, times)(body)
            else:
                pl.when(z < state["regions"] if when is None else when)(body)
        return wrap

    def wait(*copies):
        for c in copies:
            c.wait()
        untie()

    @region()
    def _():
        for c in [cp_x[0], cp_x[2], cp_qkv[Q], cp_x[1], cp_x[3], cp_qkv[K], cp_qkv[V], *cp_x[4:], *cp_o,
                  *cp_gu[0], *cp_gu[1], cp_d]:
            c.start()
        wait(cp_x[0], cp_x[2])
        load_x(0, (0, 2))
        _run(ln_pair(0, 0))
        wait(cp_qkv[Q])
        wq = prep_square(Q)
        _run(_chain(turn_square(Q), wq.take(200)))
        _run(qkv(0, 0, (Q,), pairs=(0,)), wq, ln_pair(2, 0), slack=-200)
        wait(cp_x[1], cp_x[3])
        load_x(0, (1, 3))
        _run(qkv(2, 2, (Q,), pairs=(0,)), ln_pair(0, 1), lead=300)
        _run(qkv(0, 0, (Q,), pairs=(1,)), ln_pair(2, 1), slack=-200)
        wait(cp_qkv[K], cp_qkv[V])
        _run(_chain(turn_square(K), turn_square(V)))
        wk = prep_square(K)
        _run(qkv(2, 2, (Q,), pairs=(1,)), wk.take(300), lead=250)
        k0 = qkv(0, 0, (K,))
        _run(k0.take(600), wk)
        _run(k0, prep_square(V))
        wait(*cp_x[4:], *cp_o)
        load_x(1)
        _run(turn_square(3))
        _run(qkv(0, 0, (V,), shifted=False), ln_qkv(1, 1), lead=1000, slack=50)
        _run(qkv(1, 1, (K,)), ln_qkv(3, 3), prep_square(3), slack=-200)

    @region()
    def _():
        wait(*cp_gu[0])
        preps = _chain(*[prep_gu(s) for s in range(3)])
        _run(qkv(1, 1, (Q,)), turn_gu(0), turn_gu(1), turn_gu(2), preps.take(500))
        shifts = shift(v_s, (1, 2, 3))
        _run(qkv(1, 1, (V,)), *[t for _ in range(12) for t in (shifts.take(16), preps.take(125))])
        mix = lambda att, amount: [t for i in range(4) for t in (preps.take(amount // 4), att.take(att.cost // (4 - i)))]
        _run(_chain(qkv(2, 2, (V,)), qkv(3, 3, (V,))), *mix(attention(0, values=False), 900))
        _run(_chain(qkv(2, 2, (K,)), qkv(3, 3, (K,))), *mix(attention(0, weights=False), preps.cost - TERMS2),
             o_terms(), lead=200, slack=-200)
        untie()
        _run(preps)

    late_preps = _chain(*[prep_gu(s) for s in range(3, 7)])

    @region()
    def _():
        wait(*cp_gu[1], cp_d)
        _run(_chain(*[turn_gu(s) for s in range(3, 7)], *[turn_d(t) for t in (3, 0, 1, 2)]))
        _run(proj(0), attention(1, (3,)))
        _run(qkv(3, 3, (Q,)), ln_ffn(0), lead=200)
        untie()
        _run(late_preps.take(3 * TERMS2))

    @region()
    def _():
        _run(late_preps.take(late_preps.cost - 7 * TERMS2))

    @region()
    def _():
        _run(gate_up(range(2)), prep_d1(), attention(1, (7,)))
        untie()
        _run(late_preps)

    @region(times=3)
    def _(t):
        att, prep = attention(1, range(0, EARLY, 4), g0=t), prep_d2(t)
        _run(gate_up(range(2, 6), 4 * t),
             *[p for i in range(4) for p in (prep.take(2 * TERMS2), att.take(att.cost // (4 - i)))], slack=-100)

    @pl.loop(1, 8)
    def _(m):
        before = (m - 1) & 3

        @region()
        def _():
            _run(down2(before, 0), hidden_terms(NCH - 1), attention(m, range(EARLY, 16)), o_terms())
            att = attention(m + 1, range(EARLY))
            _run(proj(m & 3), att.take(2000))
            _run(_chain(down1(before), down2(before, 2)), att.take(400), ln_ffn(m & 3))
            _run(gate_up(), att.take(300), ln_qkv(before, 0), att, slack=-150)

        @region(when=m < 5)
        def _():
            _run(qkv(m + 3, 0, (K, V, Q)))

    @region()
    def _():
        _run(_chain(down2(3, 0), down1(3)), store_out((0,), (0,)), hidden_terms(NCH - 1), store_out((0,), (1, 2, 3)),
             store_out((1, 2, 3), range(KB)), slack=800)
        for j in range(4):
            cp_out[j, 0].start()

    for k, done in ((2, (0, 1)), (3, (2,))):
        @region()
        def _():
            _run(down2(3, k, 1), store_out(range(4, NJ), done), slack=700)
            for j in range(4, NJ):
                cp_out[j, done[0]].start()

    @region()
    def _():
        _run(store_out(range(4, NJ), (3,)))
        for j in range(4, NJ):
            cp_out[j, 3].start()

    for c in cp_out.values():
        c.wait()


@jax.jit
def pallas_interleave_layers__sliding_local_dilated__glu_gated_reglu__prompt_kernel(
    A_x: jax.Array,
    A_wqkv: jax.Array,
    A_wo: jax.Array,
    B_x: jax.Array,
    B_W_gate: jax.Array,
    B_W_up: jax.Array,
    B_W_down: jax.Array,
):
    del B_x
    any_spec = pl.BlockSpec(memory_space=pl.ANY)
    out = pl.pallas_call(
        _kernel,
        out_shape=jax.ShapeDtypeStruct((L, 2 * NJ, D), BF),
        in_specs=[any_spec] * 6,
        out_specs=any_spec,
        scratch_shapes=_scratch(),
        compiler_params=pltpu.CompilerParams(
            vmem_limit_bytes=100 * 2**20, disable_semaphore_checks=True, disable_bounds_checks=True),
        name="fused_layers",
    )(A_x.reshape(L, 2 * NJ, D), A_wqkv, A_wo, B_W_gate, B_W_up, B_W_down)
    return out.reshape(1, S, D)
```

```python
import functools

import jax
import jax.numpy as jnp
import numpy as np
from jax.experimental import pallas as pl
from jax.experimental.pallas import tpu as pltpu

S, D, F = 2048, 512, 1792
DH, W = 16, 8
L = 128
NJ = 8
KB = D // L
R = 16
CH = 64
NCH = 2 * F // 4 // CH
HC = CH // 2
EPS = 1e-5
TERMS2 = 7 * 9 + 8 * 12
EARLY = 11
TUNING = dict(lag=180, lag_k=180, lag_v=180, lag_hidden=180, lag_norm=180, logit_pins=4, softmax_cost=48,
              norm_weight=1, hidden_order=tuple(range(7)), hidden_span=560)
BF, F32, U32 = jnp.bfloat16, jnp.float32, jnp.uint32
P = functools.partial


def _lo(words):
    return pltpu.bitcast(words << 16, F32)


def _hi(words):
    return pltpu.bitcast(words & np.uint32(0xFFFF0000), F32)


def _halves(words):
    return pltpu.bitcast(words, BF)


def _lanes(i, n=1):
    return pl.ds(i * n * L, n * L)


def _aligned(row):
    return row if isinstance(row, int) else pl.multiple_of(row, R)


def _add(a, b):
    return [[x + y for x, y in zip(ra, rb)] for ra, rb in zip(a, b)]


def _sub(a, b):
    return [[x - y for x, y in zip(ra, rb)] for ra, rb in zip(a, b)]


def _keep(a):
    return a


_LHS = ((_add, 0, 3), (_add, 2, 3), (_keep, 0), (_keep, 3), (_add, 0, 1), (_sub, 2, 0), (_sub, 1, 3))
_RHS = ((_add, 0, 3), (_keep, 0), (_sub, 1, 3), (_sub, 2, 0), (_keep, 3), (_add, 0, 1), (_add, 2, 3))


def _terms(table, grid):
    blocks = [[[b]] for row in grid for b in row]
    return [op(*[blocks[a] for a in args])[0][0] for op, *args in table]


def _products2(product):
    p22 = product(5)
    yield
    m3 = product(2)
    p22 = p22 + m3
    yield
    m5 = product(4)
    c12 = m3 + m5
    yield
    p11 = product(6) - m5
    yield
    m1 = product(0)
    p11, p22 = p11 + m1, p22 + m1
    yield
    m2 = product(1)
    c22 = p22 - m2
    yield
    m4 = product(3)
    yield
    return [[p11 + m4, c12], [m2 + m4, c22]]


def _products4(product, put, get, emit):
    for i in range(7):
        m = yield from _products2(lambda j: product(7 * i + j))
        for r, c in ((0, 1), (1, 1), (1, 0), (0, 0)):
            old = lambda n: get(n, 2 * r + c)
            if i < 5:
                put(i, 2 * r + c, m[r][c])
            if i == 3:
                emit(2 + r, c, m[r][c] + old(1))
            elif i == 4:
                emit(r, 2 + c, m[r][c] + old(2))
            elif i == 5:
                emit(2 + r, 2 + c, m[r][c] + (old(0) - old(1) + old(2)))
            elif i == 6:
                emit(r, c, m[r][c] + (old(0) + old(3) - old(4)))


class _Task:
    def __init__(self, cost, gen):
        self.cost, self.gen = cost, gen

    def take(self, cost):
        cost = min(cost, self.cost)
        self.cost -= cost
        if self.cost == 0:
            return _Task(cost, self.gen)

        def gen():
            done = 0
            while done < cost:
                step = next(self.gen, None)
                if step is None:
                    return
                done += step
                yield step
        return _Task(cost, gen())


def _chain(*tasks):
    def gen():
        for t in tasks:
            yield from t.gen
    return _Task(sum(t.cost for t in tasks), gen())


def _run(main, *sides, lead=0, slack=0):
    side = _chain(*sides)
    now = done = 0
    for step in main.gen:
        now += step
        while sides and done <= side.cost * (now - lead) / (main.cost - lead - slack):
            step = next(side.gen, None)
            if step is None:
                break
            done += step
    for _ in side.gen:
        pass


def _operand_layout():
    layout, row = {}, 0
    for name, (n, rows) in {**{"x%d" % s: (2, 2 * L) for s in range(4)}, "f": (7, L), "o": (2, 2 * L),
                            "h2": (7, 3 * L), "h1": (2, L)}.items():
        layout[name] = (row, rows)
        row += n * rows
    return layout, row + L


def _scratch():
    level1 = pltpu.VMEM((1, 7, 2, 2 * L, L), BF)
    return dict(
        xin=pltpu.VMEM((NJ, L, D), U32),
        wqkv_raw=pltpu.VMEM((3, D // 2, D), U32),
        wo_raw=[pltpu.VMEM((1, D // 2, L), U32)] * KB,
        wgu_raw=pltpu.VMEM((2, D // 2, F), U32),
        wd_raw=pltpu.VMEM((F // 2, D), U32),
        zero=pltpu.SMEM((2,), jnp.int32),
        turned=[[pltpu.VMEM((2, KB, L // 2, L), U32)] * 4] * 4,
        turned_ffn=[pltpu.VMEM((n, KB + 1, D // 2, L), U32) for n in (1, 1, 1, 4, 3, 1)],
        wqkv=[level1] * 3,
        wo=level1,
        wgu=pltpu.VMEM((7, 49, 1, L, L), BF),
        wd2=pltpu.VMEM((2, 49, 3, CH, L), BF),
        wd1=pltpu.VMEM((1, 7, 1, 2 * L, L), BF),
        xa=pltpu.VMEM((4, 5, D, L), F32),
        xb=pltpu.VMEM((4, 5, D, L), F32),
        stats=[pltpu.VMEM((1, 2, 8, L), F32)] * 4,
        xn=pltpu.VMEM((1, 5, D, L), F32),
        operands=[pltpu.VMEM((1, _operand_layout()[1], L), BF)] * 7,
        q_s=pltpu.VMEM((2, NJ, D, L), F32),
        k_s=pltpu.VMEM((2, 2 * NJ + 1, D, L), F32),
        v_s=pltpu.VMEM((2, 2 * NJ + 1, D, L), F32),
        probs=pltpu.VMEM((1, 16 * W, 8, L), F32),
        o_s=pltpu.VMEM((1, 5, D, L), F32),
        park_m=[pltpu.VMEM((1, 4, CH, L), F32)] * 5,
        park_h=[[pltpu.VMEM((1, 5, HC, L), F32)] * 4] * 2,
        xout=pltpu.VMEM((NJ, L, D), U32),
        sems=pltpu.SemaphoreType.DMA((36,)),
    )


def _kernel(x_hbm, wqkv_hbm, wo_hbm, wg_hbm, wu_hbm, wd_hbm, out_hbm, *,
            xin, wqkv_raw, wo_raw, wgu_raw, wd_raw, zero, turned, turned_ffn, wqkv, wo, wgu, wd2, wd1,
            xa, xb, stats, xn, operands, q_s, k_s, v_s, probs, o_s, park_m, park_h, xout, sems):
    layout, _ = _operand_layout()
    sem_ids = iter(range(sems.shape[0]))
    copy = lambda src, dst: pltpu.make_async_copy(src, dst, sems.at[next(sem_ids)])
    cp_x = [copy(x_hbm.bitcast(U32).at[:, j, :], xin.at[j]) for j in range(NJ)]
    cp_qkv = [copy(wqkv_hbm.at[:, _lanes(t, KB)], wqkv_raw.bitcast(BF).at[t]) for t in range(3)]
    cp_o = [copy(wo_hbm.at[:, _lanes(r)], wo_raw[r].bitcast(BF).at[0]) for r in range(KB)]
    cp_gu = [[copy(w.at[:, cols], wgu_raw.bitcast(BF).at[i, :, cols]) for i, w in enumerate((wg_hbm, wu_hbm))]
             for cols in (pl.ds(0, 6 * L), pl.ds(6 * L, 8 * L))]
    cp_d = copy(wd_hbm, wd_raw.bitcast(BF))
    pieces = [(j, 0, 4) for j in range(4)] + [(j, k, n) for j in range(4, NJ) for k, n in ((0, 2), (2, 1), (3, 1))]
    cp_out = {(j, k): copy(xout.at[j, :, pl.ds(k * L, n * L)], out_hbm.bitcast(U32).at[:, j, pl.ds(k * L, n * L)])
              for j, k, n in pieces}

    @pl.loop(0, 2)
    def _(i):
        zero[i] = i

    z = zero[0]
    state = dict(buffer=None, slot=0, regions=0)
    tuning = dict(TUNING)
    results = []

    def pin(*vals):
        if state["buffer"] is not None:
            for v in vals:
                state["slot"] = (state["slot"] + 1) % 8
                rows = pl.ds(operands[0].shape[1] // 2 - 8 * (state["slot"] + 1), 8)
                state["buffer"].bitcast(U32)[0, rows, :] = v if v.dtype == U32 else pltpu.bitcast(v, U32)

    def release(ref, lag="lag"):
        ready = [v for t, v in results[-64:] if t <= results[-1][0] - tuning[lag]]
        if ready:
            spare = (ref.shape[0] - 1, ref.shape[1] - 1, pl.ds(0, 8))
            ref[spare] = ready[-1] if ref.dtype == F32 else pltpu.bitcast(ready[-1], ref.dtype)

    def untie():
        results.clear()
        state["buffer"] = None

    def put(name, i, row, val):
        first, rows = layout[name]
        operands[i % 7][0, pl.ds(_aligned(first + i // 7 * rows + row), val.shape[0]), :] = val.astype(BF)

    def rhs(name, i):
        first, rows = layout[name]
        state["buffer"] = operands[i % 7]
        return _halves(operands[i % 7].bitcast(U32)[z, pl.ds((first + i // 7 * rows) // 2, rows // 2), :])

    def terms2(table, source, block, store, lag="lag", order=range(7)):
        quadrant = lambda n: [[block(2 * (n // 2) + a, 2 * (n % 2) + b) for b in range(2)] for a in range(2)]
        for i in order:
            op, *args = table[i]
            release(source(args[0]), lag)
            for n, t in enumerate(_terms(table, op(*[quadrant(a) for a in args]))):
                store(7 * i + n, t)
            yield 9 + 8 * len(args)

    def store_lhs(dst, i, k, row, t, slot=0):
        dst[slot, i, k, pl.ds(row, R), :] = t.astype(BF)
        if i % 7 == 6:
            pin(dst.bitcast(U32)[z, 0, 0, pl.ds(0, 8), :])

    def head_major(ref, lead, first, d2):
        w = ref[(*lead, pl.ds(first + d2, 8, stride=8))]
        return jnp.concatenate([_lo(w), _hi(w)], axis=0)

    def turn_square(t):
        def gen():
            for r in (0, 2, 1, 3):
                if t < 3:
                    w = _halves(wqkv_raw[t, :, _lanes(r)])
                else:
                    w = jnp.concatenate([head_major(wo_raw[r], (0,), k * L // 2, e)
                                         for k in range(KB) for e in range(L // R)]).astype(BF)
                w = pltpu.bitcast(w.T, U32)
                for k in range(KB):
                    turned[t][r][0, k] = w[:, k * L:(k + 1) * L]
                yield 30
        return _Task(4 * 30, gen())

    def prep_square(t):
        def rows(r, k, e):
            if t < 3:
                return head_major(turned[t][r], (z, k), 0, e)
            return _halves(turned[t][r][z, k, pl.ds(8 * e, 8), :]).astype(F32)

        def gen():
            for r in range(2):
                for e in range(L // R):
                    for k in range(2):
                        release(turned[t][r])
                        grid = [[rows(2 * a + r, 2 * b + k, e) for b in range(2)] for a in range(2)]
                        for i, term in enumerate(_terms(_LHS, grid)):
                            store_lhs((*wqkv, wo)[t], i, k, r * L + e * R, term)
                        yield 25
        return _Task(4 * L // R * 25, gen())

    def turned_gu(s):
        return (turned_ffn[s], 0) if s < 3 else (turned_ffn[3], s - 3)

    def turn_gu(s):
        def gen():
            dst, slot = turned_gu(s)
            for k in range(KB):
                for i in range(2):
                    w = _halves(wgu_raw[i, pl.ds(k * L // 2, L // 2), _lanes(s, 2)])
                    dst[slot, k, _lanes(i), :] = pltpu.bitcast(w.T, U32)
                    yield 32
        return _Task(8 * 32, gen())

    def prep_level2(src, block, store):
        def gen():
            for c in range(L // CH):
                for e in range(0, CH, R):
                    get = P(block, c, e) if results else functools.cache(P(block, c, e))
                    yield from terms2(_LHS, lambda _: src, get, P(store, c, e))
        return _Task(L // R * TERMS2, gen())

    def prep_gu(s):
        src, slot = turned_gu(s)

        def block(c, e, r, k):
            word, half = (4 * c + r) * HC // 2 + e // 32 * 8, e % 32 // 2
            return jnp.concatenate([
                _halves(src[z + slot, k, pl.ds(i * L + word, 8), :]).astype(F32)[half:half + 8] for i in range(2)])
        return prep_level2(src, block, lambda c, e, i, t: store_lhs(wgu, i, 0, c * CH + e, t, s))

    def turn_d(t):
        def gen():
            dst, slot = (turned_ffn[4], t) if t < 3 else (turned_ffn[5], 0)
            for k in range(4 if t < 3 else 2):
                if t < 3:
                    rows = [pl.ds(((1 + 4 * t + c) * 4 + k) * HC // 2, HC // 2) for c in range(4)]
                else:
                    rows = [pl.ds((4 * c + 2 * k) * HC // 2, HC) for c in (0, NCH - 1)]
                for n in range(2):
                    w = jnp.concatenate([wd_raw[r, _lanes(n, 2)] for r in rows], axis=0)
                    dst[slot, k, _lanes(n), :] = pltpu.bitcast(_halves(w).T, U32)
                    yield 32
        return _Task((8 if t < 3 else 4) * 32, gen())

    def prep_d2(t):
        def block(c, e, r, k):
            row = (2 * c + e // HC) * L + r * HC + e % HC
            return _halves(turned_ffn[4][z + t, k, pl.ds(row // 2, 8), :]).astype(F32)
        return prep_level2(turned_ffn[4], block, lambda c, e, i, term: store_lhs(wd2, i, t, e, term, c))

    def prep_d1():
        def gen():
            for e in range(0, 2 * L, R):
                release(turned_ffn[5])
                grid = [[_halves(turned_ffn[5][z, k, pl.ds(L * r + e // 2, 8), :]).astype(F32)
                         for k in range(2)] for r in range(2)]
                for i, term in enumerate(_terms(_LHS, grid)):
                    store_lhs(wd1, i, 0, e, term)
                yield 17
        return _Task(2 * L // R * 17, gen())

    def load_x(half, columns=(0, 2, 1, 3)):
        for c in columns:
            for k in range(KB):
                t = xin[4 * half + c, :, _lanes(k)].T
                xa[half, c, _lanes(k), :] = _lo(t)
                xa[2 + half, c, _lanes(k), :] = _hi(t)

    def store_out(columns, strips):
        def gen():
            for j in columns:
                for k in strips:
                    release(xa)
                    even, odd = [pltpu.bitcast(xa[z + q + j // 4, j % 4, _lanes(k), :].astype(BF).astype(F32), U32)
                                 for q in (0, 2)]
                    words = (even >> 16) | odd
                    pin(words[-8:])
                    xout[j, :, _lanes(k)] = words.T
                    yield 80
        return _Task(len(columns) * len(strips) * 80, gen())

    def rhs1(name, src, block, c):
        def gen():
            for e in range(0, 2 * L, R):
                release(src)
                grid = [[block(2 * a * L + e, 2 * b + c) for b in range(2)] for a in range(2)]
                for i, t in enumerate(_terms(_RHS, grid)):
                    put(name, 7 * c + i, e, t)
                yield 25
        return _Task(2 * L // R * 25, gen())

    def dot(a_ref, slot, i, row, rows, b):
        a = jnp.concatenate([_halves(a_ref.bitcast(U32)[slot, i, k, pl.ds(row // 2, rows // 2), :])
                             for k in range(a_ref.shape[2])], axis=1)
        res = jnp.dot(a, b, preferred_element_type=F32)
        results.append(((results[-1][0] if results else 0) + a.shape[0] * a.shape[1] // L // 4, res[:8]))
        return res

    def matmul1(a_ref, name, emit, pairs=(0, 1)):
        cycles = CH * a_ref.shape[2] // 4

        def gen():
            for r0 in range(0, 2 * L, CH):
                for c in pairs:
                    steps = _products2(lambda i: dot(a_ref, z, i, r0, CH, rhs(name, 7 * c + i)))
                    for _ in range(7):
                        next(steps)
                        yield cycles
                    try:
                        next(steps)
                    except StopIteration as stop:
                        for a, b in ((0, 1), (1, 1), (1, 0), (0, 0)):
                            emit(a * 2 * L + r0, 2 * b + c, stop.value[a][b])
        return _Task(2 * L // CH * 7 * len(pairs) * cycles, gen())

    def matmul2(a_ref, slot, row, rows, name, emit):
        def park(n, i, val):
            park_m[n][0, i, pl.ds(0, rows), :] = val

        cycles = rows * layout[name][1] // L // 4
        steps = _products4(lambda i: dot(a_ref, slot, i, row, rows, rhs(name, i)), park,
                           lambda n, i: park_m[n][z, i, pl.ds(0, rows), :], emit)
        return _Task(49 * cycles, (cycles for _ in steps))

    def moments(src, q, c):
        def gen():
            part = lambda k: src[z + q, c, _lanes(k), :].reshape(2, L // 16, 8, L)
            for k in range(KB):
                release(src)
                t = jnp.sum(part(k), axis=1)
                acc = t if k == 0 else acc + t
                pin(acc[1])
                yield 16
            mean = jnp.sum(acc[0] + acc[1], axis=0, keepdims=True) * (1.0 / D)
            for k in range(KB):
                release(src)
                d = part(k) - mean
                t = jnp.sum(d * d, axis=1)
                acc = t if k == 0 else acc + t
                pin(acc[0], acc[1])
                yield 48
            var = jnp.sum(acc[0] + acc[1], axis=0, keepdims=True) * (1.0 / D)
            for i, t in enumerate((mean, jax.lax.rsqrt(var + EPS))):
                stats[c][0, i] = jnp.broadcast_to(t, (8, L))
        return _Task(KB * 64, gen())

    def normalized(src, q, r, c, rows=R):
        x = src[z + q, c, pl.ds(r, rows), :].reshape(rows // 8, 8, L)
        return ((x - stats[c][z, 0][None]) * stats[c][z, 1][None]).reshape(rows, L)

    def ln_qkv(q, slot):
        m = [moments(xa, q, c) for c in range(4)]
        t = [rhs1("x%d" % slot, xa, P(normalized, xa, q), c) for c in range(2)]
        return _chain(m[0], m[2], m[1], t[0].take(200), m[3], t[0], t[1])

    def ln_pair(q, c):
        return _chain(moments(xa, q, c), moments(xa, q, c + 2), rhs1("x%d" % q, xa, P(normalized, xa, q), c))

    def ln_ffn(q):
        def scale(c):
            for r in range(0, D, L // 2):
                release(xb)
                t = normalized(xb, q, r, c, L // 2)
                xn[0, c, pl.ds(r, L // 2), :] = t
                pin(t[-8:])
                yield 16

        def terms():
            for e in range(0, L, R):
                for cost in terms2(_RHS, lambda _: xn, lambda k, c: xn[z, c, pl.ds(k * L + e, R), :],
                                   lambda i, t: put("f", i, e, t), "lag_norm"):
                    yield cost * tuning["norm_weight"]

        m = [moments(xb, q, c) for c in range(4)]
        n = [_Task(8 * 16, scale(c)) for c in range(4)]
        t = _Task(L // R * TERMS2 * tuning["norm_weight"], terms())
        return _chain(m[0], m[1], m[2], n[0], m[3], n[1], n[2], n[3], t)

    Q, K, V = range(3)

    def qkv(n, slot, which, shifted=True, pairs=(0, 1)):
        refs = q_s, k_s, v_s
        p, j0 = (n >> 1) & 1, 4 * (n & 1)

        def emit(t, r, c, val):
            j = j0 + c
            refs[t][p, j + NJ * (t > 0), pl.ds(r, CH), :] = val
            if shifted and t > 0 and (not isinstance(j, int) or j > 0):
                refs[t][p, j, pl.ds(r, CH), :] = pltpu.roll(val, 1, 1)

        return _chain(*[matmul1(wqkv[t], "x%d" % slot, P(emit, t), pairs) for t in which])

    def shift(ref, columns):
        def gen():
            for j in columns:
                for r in range(0, D, CH):
                    ref[0, j, pl.ds(r, CH), :] = pltpu.roll(ref[0, NJ + j, pl.ds(r, CH), :], 1, 1)
                    yield 8
        return _Task(len(columns) * D // CH * 8, gen())

    lane = jax.lax.broadcasted_iota(jnp.int32, (8, L), 1)

    def attend(n, u, weights, values, g0):
        p, c, g = (n >> 1) & 1, (0, 2, 1, 3)[u // 4], u % 4 + g0
        j = 4 * (n & 1) + c
        block = lambda ref, col, d: ref[z + p, col, pl.ds(_aligned(g * L + 8 * d), R), :].reshape(2, 8, L)
        if weights:
            logit = [None] * W
            for d in range(0, DH, 2):
                release(k_s, "lag_k")
                qv = block(q_s, j, d)
                for w in range(W):
                    t = qv * block(k_s, NJ + j - w, d)
                    logit[w] = (t[0] if d == 0 else logit[w] + t[0]) + t[1]
                pin(*[logit[(d // 2 * tuning["logit_pins"] + i) % W] for i in range(tuning["logit_pins"])])
                yield 32
            for w in range(c + 1, W):
                logit[w] = jnp.where(lane < (1 if w > c + 4 else 1 - (n & 1)), -1e9 * DH ** 0.5, logit[w])
            m = functools.reduce(jnp.maximum, logit)
            e = [jnp.exp2((t - m) * (DH ** -0.5 * np.log2(np.e))) for t in logit]
            total = (e[0] + e[1] + e[2] + e[3]) + (e[4] + e[5] + e[6] + e[7])
            inv = pl.reciprocal(total, approx=True)
            inv = inv * (2.0 - total * inv)
            e = [t * inv for t in e]
            if not values:
                for w in range(W):
                    probs[0, W * u + w] = e[w]
                inv = probs[z, 0]
            pin(inv)
            yield tuning["softmax_cost"]
        if values:
            for d in range(0, DH, 2):
                release(v_s, "lag_v")
                v = [block(v_s, NJ + j - w, d) for w in range(W)]
                if d == 0 and not weights:
                    e = [probs[z, W * u + w] for w in range(W)]
                o = functools.reduce(jnp.add, [e[w][None] * v[w] for w in range(W)])
                o_s[0, c, pl.ds(_aligned(g * L + 8 * d), R), :] = o.reshape(R, L)
                pin(o_s[z, 0, pl.ds(0, 8), :])
                yield 32

    def attention(n, units=range(16), weights=True, values=True, g0=0):
        cost = (256 + tuning["softmax_cost"]) * weights + 256 * values
        return _chain(*[_Task(cost, attend(n, u, weights, values, g0)) for u in units])

    def o_terms():
        return _chain(*[rhs1("o", o_s, lambda r, c: o_s[z, c, pl.ds(r, R), :], c) for c in range(2)])

    def residual(dst, src, q, r, c, val):
        rows = pl.ds(r, val.shape[0])
        dst[q, c, rows, :] = src[z + q, c, rows, :] + val

    def proj(q):
        return matmul1(wo, "o", P(residual, xb, xa, q))

    def glu(s, r, c, val):
        val = val.reshape(CH // 16, 2, 8, L)
        park_h[s % 2][2 * (r // 2) + c // 2][0, 2 * (r % 2) + c % 2] = (
            jnp.maximum(val[:, 0], 0.0) * val[:, 1]).reshape(HC, L)

    def hidden_terms(s, base=0):
        park = park_h[s % 2]

        def gen():
            for e in range(0, HC, R):
                block = lambda r, c: park[2 * (r // 2) + c // 2][z, 2 * (r % 2) + c % 2, pl.ds(e, R), :]
                if 0 < s < NCH - 1:
                    for _ in terms2(_RHS, lambda n: park[n], block,
                                    lambda i, t: put("h2", i, (base + s - 1) * HC + e, t),
                                    "lag_hidden", tuning["hidden_order"]):
                        yield 20
                else:
                    for k in range(2):
                        for c in range(2):
                            release(park[0])
                            grid = [[block(2 * a + k, 2 * b + c) for b in range(2)] for a in range(2)]
                            for i, t in enumerate(_terms(_RHS, grid)):
                                put("h1", 7 * c + i, (2 * (s > 0) + k) * HC + e, t)
                            yield 35
        return _Task(HC // R * 140, gen())

    def gate_up(chunks=range(NCH), base=0):
        def gen():
            for s in chunks:
                main = matmul2(wgu, z + (base >> 1) + s * CH // L, s * CH % L, CH, "f", P(glu, s))
                post = hidden_terms(s - 1, base) if s > 0 else _Task(0, iter(()))
                now = done = 0
                for step in main.gen:
                    now += step
                    while done < post.cost * (now - 224) / tuning["hidden_span"]:
                        done += next(post.gen)
                    yield step
                _run(post)
        return _Task(49 * len(chunks) * CH // 4, gen())

    def down2(q, first, n=2):
        def emit(a, b, val):
            for i in range(n):
                residual(xa, xa if first else xb, q, (first + i) * L + a * HC, b, val[i * HC:(i + 1) * HC])
        return matmul2(wd2, z + first // 2, first % 2 * HC, n * HC, "h2", emit)

    def down1(q):
        return matmul1(wd1, "h1", lambda r, c, val: residual(xa, xa if r < 2 * L else xb, q, r, c, val))

    def region(when=None, times=None, **knobs):
        def wrap(f):
            def body(*args):
                untie()
                tuning.update(TUNING, **knobs)
                f(*args)
            state["regions"] += 1
            if times:
                pl.loop(0, times)(body)
            else:
                pl.when(z < state["regions"] if when is None else when)(body)
        return wrap

    def wait(*copies):
        for c in copies:
            c.wait()
        untie()

    @region()
    def _():
        for c in [cp_x[0], cp_x[2], cp_qkv[Q], cp_x[1], cp_x[3], cp_qkv[K], cp_qkv[V], *cp_x[4:], *cp_o,
                  *cp_gu[0], *cp_gu[1], cp_d]:
            c.start()
        wait(cp_x[0], cp_x[2])
        load_x(0, (0, 2))
        _run(ln_pair(0, 0))
        wait(cp_qkv[Q])
        wq = prep_square(Q)
        _run(_chain(turn_square(Q), wq.take(200)))
        _run(qkv(0, 0, (Q,), pairs=(0,)), wq, ln_pair(2, 0), slack=-200)
        wait(cp_x[1], cp_x[3])
        load_x(0, (1, 3))
        _run(qkv(2, 2, (Q,), pairs=(0,)), ln_pair(0, 1), lead=300)
        _run(qkv(0, 0, (Q,), pairs=(1,)), ln_pair(2, 1), slack=-200)
        wait(cp_qkv[K], cp_qkv[V])
        _run(_chain(turn_square(K), turn_square(V)))
        wk = prep_square(K)
        _run(qkv(2, 2, (Q,), pairs=(1,)), wk.take(300), lead=250)
        k0 = qkv(0, 0, (K,))
        _run(k0.take(600), wk)
        _run(k0, prep_square(V))
        wait(*cp_x[4:], *cp_o)
        load_x(1)
        _run(turn_square(3))
        _run(qkv(0, 0, (V,), shifted=False), ln_qkv(1, 1), lead=1000, slack=50)
        _run(qkv(1, 1, (K,)), ln_qkv(3, 3), prep_square(3), slack=-200)

    @region(logit_pins=3, lag_k=150, softmax_cost=64)
    def _():
        wait(*cp_gu[0])
        preps = _chain(*[prep_gu(s) for s in range(3)])
        _run(qkv(1, 1, (Q,)), turn_gu(0), turn_gu(1), turn_gu(2), preps.take(500))
        shifts = shift(v_s, (1, 2, 3))
        _run(qkv(1, 1, (V,)), *[t for _ in range(12) for t in (shifts.take(16), preps.take(100))])
        mix = lambda att, amount: [t for i in range(4) for t in (preps.take(amount // 4), att.take(att.cost // (4 - i)))]
        _run(_chain(qkv(2, 2, (V,)), qkv(3, 3, (V,))), *mix(attention(0, values=False), 900))
        _run(_chain(qkv(2, 2, (K,)), qkv(3, 3, (K,))), *mix(attention(0, weights=False), preps.cost - TERMS2),
             o_terms(), lead=200, slack=-200)
        untie()
        _run(preps)

    late_preps = _chain(*[prep_gu(s) for s in range(3, 7)])

    @region(logit_pins=5, softmax_cost=32, norm_weight=1.15, lag_norm=150)
    def _():
        wait(*cp_gu[1], cp_d)
        _run(_chain(*[turn_gu(s) for s in range(3, 7)], *[turn_d(t) for t in (3, 0, 1, 2)]))
        _run(proj(0), attention(1, (3,)))
        _run(qkv(3, 3, (Q,)), ln_ffn(0), lead=200)
        untie()
        _run(late_preps.take(3 * TERMS2))

    @region()
    def _():
        _run(late_preps.take(late_preps.cost - 7 * TERMS2))

    @region(logit_pins=5, softmax_cost=32)
    def _():
        _run(gate_up(range(2)), prep_d1(), attention(1, (7,)))
        untie()
        _run(late_preps)

    @region(times=3, logit_pins=2, softmax_cost=32, lag=210, lag_k=165, lag_v=150)
    def _(t):
        att, prep = attention(1, range(0, EARLY, 4), g0=t), prep_d2(t)
        _run(gate_up(range(2, 6), 4 * t),
             *[p for i in range(4) for p in (prep.take(2 * TERMS2), att.take(att.cost // (4 - i)))],
             lead=-100, slack=-200)

    @pl.loop(1, 8)
    def _(m):
        before = (m - 1) & 3

        @region(lag_v=150, lag_hidden=210, lag_norm=195, hidden_order=(6, 2, 4, 3, 5, 1, 0), hidden_span=590)
        def _():
            _run(down2(before, 0), hidden_terms(NCH - 1), attention(m, range(EARLY, 16)), o_terms())
            att = attention(m + 1, range(EARLY))
            _run(proj(m & 3), att.take(2000))
            _run(_chain(down1(before), down2(before, 2)), att.take(400), ln_ffn(m & 3))
            _run(gate_up(), att.take(200), ln_qkv(before, 0), att, slack=-150)

        @region(when=m < 5)
        def _():
            _run(qkv(m + 3, 0, (K, V, Q)))

    @region()
    def _():
        _run(_chain(down2(3, 0), down1(3)), store_out((0,), (0,)), hidden_terms(NCH - 1), store_out((0,), (1, 2, 3)),
             store_out((1, 2, 3), range(KB)), slack=800)
        for j in range(4):
            cp_out[j, 0].start()

    for k, done in ((2, (0, 1)), (3, (2,))):
        @region()
        def _():
            _run(down2(3, k, 1), store_out(range(4, NJ), done), slack=700)
            for j in range(4, NJ):
                cp_out[j, done[0]].start()

    @region()
    def _():
        _run(store_out(range(4, NJ), (3,)))
        for j in range(4, NJ):
            cp_out[j, 3].start()

    for c in cp_out.values():
        c.wait()


@jax.jit
def pallas_interleave_layers__sliding_local_dilated__glu_gated_reglu__prompt_kernel(
    A_x: jax.Array,
    A_wqkv: jax.Array,
    A_wo: jax.Array,
    B_x: jax.Array,
    B_W_gate: jax.Array,
    B_W_up: jax.Array,
    B_W_down: jax.Array,
):
    del B_x
    any_spec = pl.BlockSpec(memory_space=pl.ANY)
    out = pl.pallas_call(
        _kernel,
        out_shape=jax.ShapeDtypeStruct((L, 2 * NJ, D), BF),
        in_specs=[any_spec] * 6,
        out_specs=any_spec,
        scratch_shapes=_scratch(),
        compiler_params=pltpu.CompilerParams(
            vmem_limit_bytes=100 * 2**20, disable_semaphore_checks=True, disable_bounds_checks=True),
        name="fused_layers",
    )(A_x.reshape(L, 2 * NJ, D), A_wqkv, A_wo, B_W_gate, B_W_up, B_W_down)
    return out.reshape(1, S, D)
```
